```python
import os as _os
_os.environ.setdefault("JAX_PLATFORMS", "cpu")
import jax
import jax.numpy as jnp

def _softmax(x, axis=-1):
    return jax.nn.softmax(x, axis=axis)
def _gelu(x):
    return jax.nn.gelu(x, approximate=True)
def _silu(x):
    return jax.nn.silu(x)
def _sigmoid(x):
    return jax.nn.sigmoid(x)
def _layernorm(x, axis=-1, eps=1e-5):
    m = jnp.mean(x, axis=axis, keepdims=True)
    v = jnp.var(x, axis=axis, keepdims=True)
    return (x - m) / jnp.sqrt(v + eps)
def _scatter_add(tgt, idx, src, axis=0):
    return tgt.at[idx].add(src)
def _segment_sum(src, seg, n):
    return jax.ops.segment_sum(src, seg, n)
class _Rng:
    def __init__(self, key):
        self._k = key
    def _next(self):
        self._k, sub = jax.random.split(self._k)
        return sub
    def normal(self, shape):
        return jax.random.normal(self._next(), shape, dtype=jnp.bfloat16)
    def randint(self, lo, hi, shape):
        return jax.random.randint(self._next(), shape, lo, hi, dtype=jnp.int32)
    def uniform(self, shape, lo=0.0, hi=1.0):
        return jax.random.uniform(self._next(), shape, jnp.bfloat16, lo, hi)
    def permutation(self, n):
        return jax.random.permutation(self._next(), n)


kernel_name = 'sequential_preLN__linear_attn_block__dense_activation_squared_relu__prompt'

def setup_inputs():
    _rng = _Rng(jax.random.key(int.from_bytes(__import__("os").urandom(4), "little")))
    _w = (lambda a: (lambda t: t.astype(jnp.bfloat16) if jnp.issubdtype(t.dtype, jnp.floating) else t)(jnp.asarray(a)))
    def _A_setup():
        B, S, D = 1, 2048, 576
        return {
            "x": _w((lambda *s: _rng.normal(s) * 0.05)(B, S, D)),
            "wqkv": _w((lambda *s: _rng.normal(s) * 0.1)(D, 3 * D)),
            "wo": _w((lambda *s: _rng.normal(s) * 0.05)(D, D)),
        }
    _A_in = _A_setup()

    def _B_setup():
        B, S, D, F = 1, 2048, 576, 4608
        return {
            "x": _w((lambda *s: _rng.normal(s) * 0.05)(B, S, D)),
            "w1": _w((lambda *s: _rng.normal(s) * 0.05)(D, F)),
            "b1": _w((lambda *s: _rng.normal(s) * 0.05)(F)),
            "w2": _w((lambda *s: _rng.normal(s) * 0.05)(F, D)),
            "b2": _w((lambda *s: _rng.normal(s) * 0.05)(D)),
        }
    _B_in = _B_setup()

    return {
        "A_x": _A_in["x"],
        "A_wqkv": _A_in["wqkv"],
        "A_wo": _A_in["wo"],
        "B_x": _B_in["x"],
        "B_w1": _B_in["w1"],
        "B_b1": _B_in["b1"],
        "B_w2": _B_in["w2"],
        "B_b2": _B_in["b2"],
    }

def reference(A_x, A_wqkv, A_wo, B_x, B_w1, B_b1, B_w2, B_b2):
    def _A_ref(x, wqkv, wo):
        B, S, D = x.shape
        H = 32; Dh = D // H
        qkv = (lambda x, *d: x.transpose(*d))((x @ wqkv).reshape(B, S, 3, H, Dh), 2, 0, 3, 1, 4)
        q, k, v = qkv[0], qkv[1], qkv[2]
        phi = lambda t: jnp.where(t > 0, t + 1, jnp.exp(t)) + 1e-6
        pq, pk = phi(q), phi(k)
        kv = jnp.einsum("bhsd,bhse->bhde", pk, v)
        z = jnp.einsum("bhsd->bhd", pk)
        num = jnp.einsum("bhqd,bhde->bhqe", pq, kv)
        den = jnp.einsum("bhqd,bhd->bhq", pq, z)[..., None] + 1e-6
        o = num / den
        return (lambda x, *d: x.transpose(*d))(o, 0, 2, 1, 3).reshape(B, S, D) @ wo

    def _B_ref(x, w1, b1, w2, b2):
        h = jnp.einsum("bsd,df->bsf", x, w1) + b1
        zero = jnp.zeros_like(h)
        r = jnp.where(h > zero, h, zero)
        h = r * r
        out = jnp.einsum("bsf,fd->bsd", h, w2) + b2
        return out

    x = A_x
    h = x + _A_ref(_layernorm(x, axis=-1), A_wqkv, A_wo)
    h2 = h + _B_ref(_layernorm(h, axis=-1), B_w1, B_b1, B_w2, B_b2)
    return h2
```

```python
import jax
import jax.numpy as jnp
import jax.experimental.pallas as pl
import jax.experimental.pallas.tpu as pltpu

H = 32
LANES = 128
NT = (((1,), (1,)), ((), ()))


def _div_const(x, d):
    m = (65536 + d - 1) // d
    return jnp.right_shift(x * m, 16)


def _ln_t(x, eps=1e-5):
    m = jnp.mean(x, axis=0, keepdims=True)
    xc = x - m
    v = jnp.mean(xc * xc, axis=0, keepdims=True)
    return xc * jax.lax.rsqrt(v + eps)


def _phi(t):
    return jnp.where(t > 0, t + 1.0, jnp.exp(t)) + 1e-6


def _make_kernel(S, D, F, T, FC, QS):
    DH = D // H
    NT_D = -(-D // LANES)
    NB = S // T
    NC = F // FC
    NL = T // LANES
    WCH = NT_D * LANES
    NWCH = -(-3 * D // WCH)

    def tile_window(j):
        lo = j * LANES
        hi = min(D, lo + LANES)
        h_lo = lo // DH
        h_hi = (hi - 1) // DH
        rlo = (h_lo * DH) // 16 * 16
        rhi = min(D, -(-((h_hi + 1) * DH) // 16) * 16)
        return lo, hi, rlo, rhi

    WINS = [tile_window(j) for j in range(NT_D)]
    WMAX = max(w[3] - w[2] for w in WINS)

    def head_mask(j):
        lo, hi, rlo, rhi = WINS[j]
        shp = (rhi - rlo, hi - lo)
        r = jax.lax.broadcasted_iota(jnp.int32, shp, 0) + rlo
        c = jax.lax.broadcasted_iota(jnp.int32, shp, 1) + lo
        return _div_const(r, DH) == _div_const(c, DH)

    def overlap_add(parts):
        pieces = []
        pos = 0
        for j, part in enumerate(parts):
            rlo, rhi = WINS[j][2], WINS[j][3]
            nxt = WINS[j + 1][2] if j + 1 < len(parts) else rhi
            if pos < nxt:
                pieces.append(part[pos - rlo:nxt - rlo])
            if j + 1 < len(parts):
                pieces.append(part[nxt - rlo:rhi - rlo] + parts[j + 1][:rhi - nxt])
                pos = rhi
        return jnp.concatenate(pieces, axis=0)

    def kernel(xt_hbm, wqkv_hbm, b1_ref, b2_ref, wo_hbm, w1_hbm, w2t_hbm, o_hbm,
               x_ref, wqkv_ref, wt_ref, pqt_ref, kv_ref, z_ref, mt_ref, b2c_ref,
               wo_ref, w1_ref, w2t_ref, ob_ref, tmp_ref, zp_ref, nxt_ref,
               sem_x, sem_w, sem_big, sem_o):

        def x_copy(b):
            return pltpu.make_async_copy(xt_hbm.at[:, pl.ds(b * T, T)],
                                         x_ref.at[b], sem_x.at[b])

        def w_copy(c):
            lo = c * WCH
            n = min(3 * D, lo + WCH) - lo
            return pltpu.make_async_copy(wqkv_hbm.at[:, pl.ds(lo, n)],
                                         wqkv_ref.at[:, pl.ds(lo, n)], sem_w.at[c])

        def big_copies():
            return (pltpu.make_async_copy(wo_hbm, wo_ref, sem_big.at[0]),
                    pltpu.make_async_copy(w1_hbm, w1_ref, sem_big.at[1]),
                    pltpu.make_async_copy(w2t_hbm, w2t_ref, sem_big.at[2]))

        def o_copy(b, l):
            off = b * T + l * LANES
            if not isinstance(b, int):
                off = pl.multiple_of(off, LANES)
            return pltpu.make_async_copy(ob_ref.at[b, :, pl.ds(l * LANES, LANES)],
                                         o_hbm.at[:, pl.ds(off, LANES)],
                                         sem_o.at[b * NL + l])

        w_copy(0).start()
        x_copy(0).start()

        kv_ref[...] = jnp.zeros_like(kv_ref)
        z_ref[...] = jnp.zeros_like(z_ref)
        b2 = b2_ref[...].reshape(1, D)
        b2 = jnp.broadcast_to(b2.astype(jnp.float32), (LANES, D))
        b2c_ref[...] = b2.T

        def tmp_store(row0, val):
            n = val.shape[0]
            for ct in range(NT_D):
                lo = ct * LANES
                hi = min(D, lo + LANES)
                piece = val[:, lo:hi]
                if hi - lo < LANES:
                    piece = jnp.concatenate(
                        [piece, jnp.zeros((n, LANES - (hi - lo)), val.dtype)], axis=1)
                tmp_ref[ct, row0:row0 + n, :] = piece

        def tmp_rows(d):
            out = jnp.concatenate(
                [tmp_ref[ct, pl.ds(d, H, stride=DH), :] for ct in range(NT_D)], axis=1)
            return out[:, :D]

        def transpose_w(c):
            for t in range(NT_D):
                lo = c * WCH + t * LANES
                hi = min(3 * D, lo + LANES)
                if lo >= hi:
                    continue
                w = wqkv_ref[:, lo:hi].astype(jnp.float32).T
                if lo < D:
                    nq = min(hi, D) - lo
                    tmp_store(lo, w[:nq])
                    if lo + nq < hi:
                        wt_ref[lo + nq:hi, :] = w[nq:].astype(jnp.bfloat16)
                else:
                    wt_ref[lo:hi, :] = w.astype(jnp.bfloat16)
            if c == 0:
                for d in range(DH):
                    wt_ref[d * H:(d + 1) * H, :] = tmp_rows(d).astype(jnp.bfloat16)

        def phase0(b, first):
            if first:
                w_copy(0).wait()
                transpose_w(0)
                x_copy(b).wait()
                for cc in range(1, NWCH):
                    w_copy(cc).start()
            xn = _ln_t(x_ref[b].astype(jnp.float32)).astype(jnp.bfloat16)
            if first:
                q = jnp.dot(wt_ref[:QS, :], xn, preferred_element_type=jnp.float32)
                pqt_ref[b, :QS, :] = _phi(q).astype(jnp.bfloat16)
                for cc in range(1, NWCH):
                    w_copy(cc).wait()
                for bb in range(1, NB):
                    x_copy(bb).start()
                q = jnp.dot(wt_ref[QS:D, :], xn, preferred_element_type=jnp.float32)
                pqt_ref[b, QS:, :] = _phi(q).astype(jnp.bfloat16)
                for cc in range(1, NWCH):
                    transpose_w(cc)
            else:
                q = jnp.dot(wt_ref[:D, :], xn, preferred_element_type=jnp.float32)
                pqt_ref[b] = _phi(q).astype(jnp.bfloat16)
            k = jnp.dot(wt_ref[D:2 * D, :], xn, preferred_element_type=jnp.float32)
            pk = _phi(k)
            zs = pk[:, :LANES]
            for l in range(1, NL):
                zs = zs + pk[:, l * LANES:(l + 1) * LANES]
            z_ref[...] += zs
            pk = pk.astype(jnp.bfloat16)
            v = jnp.dot(wt_ref[2 * D:, :], xn, preferred_element_type=jnp.float32)
            v = v.astype(jnp.bfloat16)
            for j in range(NT_D):
                lo, hi, rlo, rhi = WINS[j]
                kv = jax.lax.dot_general(pk[rlo:rhi, :], v[lo:hi, :], NT,
                                         preferred_element_type=jnp.float32)
                kv_ref[j, :rhi - rlo, :hi - lo] += kv
            if first:
                for bb in range(1, NB):
                    x_copy(bb).wait()
                for cc in big_copies():
                    cc.start()

        phase0(0, True)

        def body0(b, carry):
            phase0(b, False)
            return carry
        jax.lax.fori_loop(1, NB, body0, 0)

        def scaled_pq(b):
            pq = pqt_ref[b].astype(jnp.float32)
            zt = jnp.concatenate([zp_ref[...]] * NL, axis=1)
            pz = pq * zt
            den = pz[:H]
            for d in range(1, DH):
                den = den + pz[d * H:(d + 1) * H]
            rr = 1.0 / (den + 1e-6)
            return jnp.concatenate(
                [(pq[d * H:(d + 1) * H] * rr).astype(jnp.bfloat16) for d in range(DH)],
                axis=0)

        for c in big_copies():
            c.wait()
        parts = []
        for j in range(NT_D):
            lo, hi, rlo, rhi = WINS[j]
            kv = jnp.where(head_mask(j), kv_ref[j, :rhi - rlo, :hi - lo], 0.0)
            parts.append(jnp.dot(kv.astype(jnp.bfloat16), wo_ref[lo:hi, :],
                                 preferred_element_type=jnp.float32))
        tmp_store(0, overlap_add(parts))
        m = jnp.concatenate([tmp_rows(d) for d in range(DH)], axis=0)
        mt_ref[...] = m.T.astype(jnp.bfloat16)
        z = jnp.sum(z_ref[...], axis=1, keepdims=True)
        z_ref[...] = jnp.broadcast_to(z, z_ref.shape)
        for d in range(DH):
            zp_ref[d * H:(d + 1) * H, :] = z_ref[pl.ds(d, H, stride=DH), :]
        nxt_ref[0] = scaled_pq(0)

        def body1(b, carry):
            pqs = nxt_ref[b % 2]
            attn = jnp.dot(mt_ref[...], pqs, preferred_element_type=jnp.float32)
            h = x_ref[b].astype(jnp.float32) + attn
            hn = _ln_t(h).T.astype(jnp.bfloat16)
            acc = h + jnp.concatenate([b2c_ref[...]] * NL, axis=1)
            b1 = b1_ref[...].reshape(1, F)
            for c in range(NC):
                f = jnp.dot(hn, w1_ref[:, c * FC:(c + 1) * FC],
                            preferred_element_type=jnp.float32)
                f = f + b1[:, c * FC:(c + 1) * FC].astype(jnp.float32)
                f = jnp.maximum(f, 0.0)
                f = (f * f).astype(jnp.bfloat16)
                if c == 0:
                    nxt_ref[(b + 1) % 2] = scaled_pq(jnp.minimum(b + 1, NB - 1))
                if c + 1 < NC:
                    acc = acc + jax.lax.dot_general(
                        w2t_ref[:, c * FC:(c + 1) * FC], f, NT,
                        preferred_element_type=jnp.float32)
                else:
                    for l in range(NL):
                        a = acc[:, l * LANES:(l + 1) * LANES] + jax.lax.dot_general(
                            w2t_ref[:, c * FC:(c + 1) * FC],
                            f[l * LANES:(l + 1) * LANES], NT,
                            preferred_element_type=jnp.float32)
                        ob_ref[b, :, l * LANES:(l + 1) * LANES] = a.astype(ob_ref.dtype)
                        o_copy(b, l).start()
            return carry
        jax.lax.fori_loop(0, NB, body1, 0)

        for b in range(NB):
            for l in range(NL):
                o_copy(b, l).wait()

    scratch = [
        pltpu.VMEM((NB, D, T), jnp.bfloat16),
        pltpu.VMEM((D, 3 * D), jnp.bfloat16),
        pltpu.VMEM((3 * D, D), jnp.bfloat16),
        pltpu.VMEM((NB, D, T), jnp.bfloat16),
        pltpu.VMEM((NT_D, WMAX, LANES), jnp.float32),
        pltpu.VMEM((D, LANES), jnp.float32),
        pltpu.VMEM((D, D), jnp.bfloat16),
        pltpu.VMEM((D, LANES), jnp.float32),
        pltpu.VMEM((D, D), jnp.bfloat16),
        pltpu.VMEM((D, F), jnp.bfloat16),
        pltpu.VMEM((D, F), jnp.bfloat16),
        pltpu.VMEM((NB, D, T), jnp.bfloat16),
        pltpu.VMEM((NT_D, D, LANES), jnp.float32),
        pltpu.VMEM((D, LANES), jnp.float32),
        pltpu.VMEM((2, D, T), jnp.bfloat16),
        pltpu.SemaphoreType.DMA((NB,)),
        pltpu.SemaphoreType.DMA((NWCH,)),
        pltpu.SemaphoreType.DMA((3,)),
        pltpu.SemaphoreType.DMA((NB * NL,)),
    ]
    return kernel, scratch


@jax.jit
def pallas_sequential_preLN__linear_attn_block__dense_activation_squared_relu__prompt_kernel(
    A_x: jax.Array,
    A_wqkv: jax.Array,
    A_wo: jax.Array,
    B_x: jax.Array,
    B_w1: jax.Array,
    B_b1: jax.Array,
    B_w2: jax.Array,
    B_b2: jax.Array,
):
    B, S, D = A_x.shape
    F = B_w1.shape[1]
    assert B == 1
    kernel, scratch = _make_kernel(S, D, F, T=512, FC=1152, QS=544)
    out_t = pl.pallas_call(
        kernel,
        in_specs=[
            pl.BlockSpec(memory_space=pl.ANY),
            pl.BlockSpec(memory_space=pl.ANY),
            pl.BlockSpec(memory_space=pltpu.VMEM),
            pl.BlockSpec(memory_space=pltpu.VMEM),
            pl.BlockSpec(memory_space=pl.ANY),
            pl.BlockSpec(memory_space=pl.ANY),
            pl.BlockSpec(memory_space=pl.ANY),
        ],
        out_specs=pl.BlockSpec(memory_space=pl.ANY),
        out_shape=jax.ShapeDtypeStruct((D, S), A_x.dtype),
        scratch_shapes=scratch,
        compiler_params=pltpu.CompilerParams(vmem_limit_bytes=100 * 1024 * 1024),
    )(A_x.reshape(S, D).T, A_wqkv, B_b1, B_b2, A_wo, B_w1, B_w2.T)
    return out_t.T.reshape(B, S, D)
```
